```python
import os as _os
_os.environ.setdefault("JAX_PLATFORMS", "cpu")
import jax
import jax.numpy as jnp

def _softmax(x, axis=-1):
    return jax.nn.softmax(x, axis=axis)
def _gelu(x):
    return jax.nn.gelu(x, approximate=True)
def _silu(x):
    return jax.nn.silu(x)
def _sigmoid(x):
    return jax.nn.sigmoid(x)
def _layernorm(x, axis=-1, eps=1e-5):
    m = jnp.mean(x, axis=axis, keepdims=True)
    v = jnp.var(x, axis=axis, keepdims=True)
    return (x - m) / jnp.sqrt(v + eps)
def _scatter_add(tgt, idx, src, axis=0):
    return tgt.at[idx].add(src)
def _segment_sum(src, seg, n):
    return jax.ops.segment_sum(src, seg, n)
class _Rng:
    def __init__(self, key):
        self._k = key
    def _next(self):
        self._k, sub = jax.random.split(self._k)
        return sub
    def normal(self, shape):
        return jax.random.normal(self._next(), shape, dtype=jnp.bfloat16)
    def randint(self, lo, hi, shape):
        return jax.random.randint(self._next(), shape, lo, hi, dtype=jnp.int32)
    def uniform(self, shape, lo=0.0, hi=1.0):
        return jax.random.uniform(self._next(), shape, jnp.bfloat16, lo, hi)
    def permutation(self, n):
        return jax.random.permutation(self._next(), n)


kernel_name = 'parallel_sum__mha_block_cached__dense_activation_mish__decode'

def setup_inputs():
    _rng = _Rng(jax.random.key(int.from_bytes(__import__("os").urandom(4), "little")))
    _w = (lambda a: (lambda t: t.astype(jnp.bfloat16) if jnp.issubdtype(t.dtype, jnp.floating) else t)(jnp.asarray(a)))
    def _A_setup():
        B, Sq, D = 1, 1, 448
        H, Sk, Dh = 16, 16384, 256
        return {
            "x": _w((lambda *s: _rng.normal(s) * 0.05)(B, Sq, D)),
            "k_cache": _w((lambda *s: _rng.normal(s) * 1.6)(B, H, Sk, Dh)),
            "v_cache": _w((lambda *s: _rng.normal(s) * 0.8)(B, H, Sk, Dh)),
            "wq": _w((lambda *s: _rng.normal(s) * 1.6)(D, H * Dh) * (D ** -0.5)),
            "wo": _w((lambda *s: _rng.normal(s) * 0.8)(H * Dh, D) * ((H * Dh) ** -0.5)),
        }
    _A_in = _A_setup()

    def _B_setup():
        B, S, D, F = 1, 1, 448, 1792
        return {
            "x": _w((lambda *s: _rng.normal(s) * 0.05)(B, S, D)),
            "w1": _w((lambda *s: _rng.normal(s) * 0.8)(D, F) * (D ** -0.5)),
            "b1": _w((lambda *s: _rng.normal(s) * 0.05)(F)),
            "w2": _w((lambda *s: _rng.normal(s) * 0.05)(F, D) * (F ** -0.5)),
        }
    _B_in = _B_setup()

    return {
        "A_x": _A_in["x"],
        "A_k_cache": _A_in["k_cache"],
        "A_v_cache": _A_in["v_cache"],
        "A_wq": _A_in["wq"],
        "A_wo": _A_in["wo"],
        "B_x": _B_in["x"],
        "B_w1": _B_in["w1"],
        "B_b1": _B_in["b1"],
        "B_w2": _B_in["w2"],
    }

def reference(A_x, A_k_cache, A_v_cache, A_wq, A_wo, B_x, B_w1, B_b1, B_w2):
    def _A_ref(x, k_cache, v_cache, wq, wo):
        B, Sq, D = x.shape
        H, Dh = 16, 256
        q = (lambda x, *d: x.transpose(*d))((x @ wq).reshape(B, Sq, H, Dh), 0, 2, 1, 3)
        scores = jnp.einsum("bhqd,bhkd->bhqk", q, k_cache) * (Dh ** -0.5)
        p = _softmax(scores, axis=-1)
        o = jnp.einsum("bhqk,bhkd->bhqd", p, v_cache)
        return (lambda x, *d: x.transpose(*d))(o, 0, 2, 1, 3).reshape(B, Sq, H * Dh) @ wo

    def _B_ref(x, w1, b1, w2):
        h = jnp.einsum("bsd,df->bsf", x, w1) + b1
        sp = jnp.log1p(jnp.exp(-jnp.abs(h))) + jnp.where(h > 0, h, jnp.zeros_like(h))
        act = h * jnp.tanh(sp)
        return jnp.einsum("bsf,fd->bsd", act, w2)

    x = A_x
    xn = _layernorm(x, axis=-1)
    return x + _A_ref(xn, A_k_cache, A_v_cache, A_wq, A_wo) + _B_ref(xn, B_w1, B_b1, B_w2)
```

```python
import functools

import jax
import jax.numpy as jnp
from jax import lax
from jax.experimental import pallas as pl
from jax.experimental.pallas import tpu as pltpu

F32 = jnp.float32
BF16 = jnp.bfloat16
NT = (((1,), (1,)), ((), ()))


def _nt(a, b):
    return lax.dot_general(a, b, NT, preferred_element_type=F32)


def _nn(a, b):
    return jnp.dot(a, b, preferred_element_type=F32)


def make(R=128, D=4, interleave=True, checks=False, semchecks=True, piece=64, compute=True):
    def fn(A_x, A_k_cache, A_v_cache, A_wq, A_wo, B_x, B_w1, B_b1, B_w2):
        _, _, DM = A_x.shape
        _, H, SK, DH = A_k_cache.shape
        FF = B_w1.shape[1]
        HD = H * DH
        NS = SK // R
        NP = R // piece
        G = H * NP
        SLOTS = D + 1

        def kernel(x_hbm, k_hbm, v_hbm, wq_hbm, wo_hbm, w1_hbm, b1_hbm, w2_hbm, o_hbm,
                   x_v, b1_v, o_v, wq_v, wo_v, w1_v, w2_v, ring, s_v, rsem, wsem):
            row = lax.broadcasted_iota(jnp.int32, (H, 128), 0)

            def kv_copy(src, step, slot, j):
                h, p = j % H, j // H
                r0 = step * R + p * piece
                if not isinstance(r0, int):
                    r0 = pl.multiple_of(r0, piece)
                return pltpu.make_async_copy(
                    src.at[0, h, pl.ds(r0, piece)],
                    ring.at[slot, h, pl.ds(p * piece, piece)], rsem.at[slot])

            def wait_all(buf, sem):
                pltpu.make_async_copy(buf, buf, sem).wait()

            def w_copies(src, dst, sem, r_lo, r_hi, c_lo, c_hi, cw):
                out = []
                for r in range(r_lo, r_hi, 8):
                    for c in range(c_lo, c_hi, cw):
                        idx = (pl.ds(r, 8), pl.ds(c, cw))
                        out.append(pltpu.make_async_copy(src.at[idx], dst.at[idx], sem))
                return out

            def spread(lst, n=16):
                m = -(-len(lst) // n)
                return [lst[a * m + b] for b in range(m) for a in range(n) if a * m + b < len(lst)]

            class Issuer:
                def __init__(self, copies):
                    self.copies = list(copies)
                    self.n = 0

                def issue(self, count):
                    for _ in range(count):
                        if self.n < len(self.copies):
                            self.copies[self.n].start(priority=self.n % 2)
                            self.n += 1

                def rest(self):
                    self.issue(len(self.copies))

            cx = pltpu.make_async_copy(x_hbm, x_v, wsem.at[0])
            cb = pltpu.make_async_copy(b1_hbm, b1_v, wsem.at[1])
            cx.start()
            cb.start()
            pro = Issuer(
                spread(w_copies(wq_hbm, wq_v, wsem.at[2], 0, DM, 0, HD, 2048))
                + spread(w_copies(w1_hbm, w1_v, wsem.at[3], 0, DM, 0, FF, FF))
                + [kv_copy(k_hbm, s, s, j) for s in range(D) for j in range(G)])
            pro.issue(112)
            cx.wait()
            x = x_v[0].astype(F32)
            mean = jnp.mean(x, axis=-1, keepdims=True)
            xc = x - mean
            var = jnp.mean(xc * xc, axis=-1, keepdims=True)
            xn = xc / jnp.sqrt(var + 1e-5)
            xn = jnp.broadcast_to(xn, (H, DM)).astype(BF16)
            pro.issue(56 + 24)
            wait_all(wq_v, wsem.at[2])
            row2 = lax.broadcasted_iota(jnp.int32, (H, DH), 0)
            q = jnp.zeros((H, DH), F32)
            for h in range(H):
                pro.issue(4)
                q = jnp.where(row2 == h, _nn(xn, wq_v[:, h * DH:(h + 1) * DH]), q)
            q = (q * (DH ** -0.5)).astype(BF16)
            wait_all(w1_v, wsem.at[3])
            cb.wait()
            b1 = b1_v[...].astype(F32)
            acts = []
            for c in range(FF // 128):
                pro.issue(2)
                hh = _nn(xn, w1_v[:, c * 128:(c + 1) * 128]) + b1[c:c + 1, :]
                sp = jnp.log1p(jnp.exp(-jnp.abs(hh))) + jnp.where(hh > 0, hh, 0.0)
                acts.append((hh * jnp.tanh(sp)).astype(BF16))
            act = jnp.concatenate(acts, axis=1)
            pro.rest()

            rowr = lax.broadcasted_iota(jnp.int32, (H, R), 0)

            def nxt(slot):
                return jnp.where(slot == SLOTS - 1, 0, slot + 1)

            def k_step(i, slot, m, issue):
                wait_all(ring.at[slot], rsem.at[slot])
                if not interleave:
                    issue(G)
                s = jnp.zeros((H, R), F32)
                for h in range(H):
                    if interleave:
                        issue(NP)
                    if compute:
                        s = jnp.where(rowr == h, _nt(q, ring[slot, h]), s)
                s_v[i] = s
                return jnp.maximum(m, s)

            def v_step(i, slot, mx, l, acc, issue):
                wait_all(ring.at[slot], rsem.at[slot])
                if not interleave:
                    issue(G)
                p = jnp.exp(s_v[i] - mx)
                pb = p.astype(BF16)
                t = jnp.zeros((H, DH), F32)
                for h in range(H):
                    if interleave:
                        issue(NP)
                    if compute:
                        t = jnp.where(row2 == h, _nn(pb, ring[slot, h]), t)
                return l + p, acc + t

            def k_body(src, base):
                def body(i, c):
                    slot, prev, m = c
                    iss = Issuer([kv_copy(src, i + base, prev, j) for j in range(G)])
                    m = k_step(i, slot, m, iss.issue)
                    return nxt(slot), slot, m
                return body

            c = (0, SLOTS - 1, jnp.full((H, R), -jnp.inf, F32))
            c = lax.fori_loop(0, NS - D, k_body(k_hbm, D), c)
            slot, prev, m = lax.fori_loop(NS - D, NS, k_body(v_hbm, D - NS), c)
            mx = jnp.broadcast_to(jnp.max(m, axis=1, keepdims=True), (H, R))

            def v_body(i, c):
                slot, prev, l, acc = c
                iss = Issuer([kv_copy(v_hbm, i + D, prev, j) for j in range(G)])
                l, acc = v_step(i, slot, mx, l, acc, iss.issue)
                return nxt(slot), slot, l, acc

            c = (slot, prev, jnp.zeros((H, R), F32), jnp.zeros((H, DH), F32))
            _, _, l, acc = lax.fori_loop(0, NS - D, v_body, c)

            blocks = [(r, min(r + 128, DM), cc, cc + 2048) for r in range(0, DM, 128) for cc in (0, 2048)]
            epi = spread(w_copies(w2_hbm, w2_v, wsem.at[4], 0, DM, 0, FF, FF))
            for n, (r0, r1, c0, c1) in enumerate(blocks):
                epi += w_copies(wo_hbm, wo_v, wsem.at[5 + n], r0, r1, c0, c1, 2048)
            epi = Issuer(epi)
            for i in range(NS - D, NS):
                l, acc = v_step(i, (NS + i) % SLOTS, mx, l, acc, epi.issue)
            epi.issue(8)
            o = (acc / jnp.sum(l, axis=1, keepdims=True))
            ob = jnp.concatenate(
                [jnp.broadcast_to(o[h:h + 1, :], (H, DH)) for h in range(H)], axis=1).astype(BF16)
            wait_all(w2_v, wsem.at[4])
            outs = []
            for r in range(0, DM, 128):
                epi.issue(8)
                r1 = min(r + 128, DM)
                outs.append(x[:, r:r1] + _nt(act, w2_v[r:r1, :])[0:1])
            epi.rest()
            for n, (r0, r1, c0, c1) in enumerate(blocks):
                blk = wo_v.at[pl.ds(r0, r1 - r0), pl.ds(c0, c1 - c0)]
                wait_all(blk, wsem.at[5 + n])
                outs[r0 // 128] += _nt(ob[:, c0:c1], wo_v[r0:r1, c0:c1])[0:1]
            o_v[0] = jnp.concatenate(outs, axis=1).astype(BF16)
            co = pltpu.make_async_copy(o_v, o_hbm, wsem.at[0])
            co.start()
            co.wait()

        hbm = pl.BlockSpec(memory_space=pltpu.HBM)
        return pl.pallas_call(
            kernel,
            out_shape=jax.ShapeDtypeStruct(A_x.shape, A_x.dtype),
            in_specs=[hbm] * 8,
            out_specs=hbm,
            scratch_shapes=[
                pltpu.VMEM(A_x.shape, BF16),
                pltpu.VMEM((FF // 128, 128), BF16),
                pltpu.VMEM(A_x.shape, BF16),
                pltpu.VMEM((DM, HD), BF16),
                pltpu.VMEM((DM, HD), BF16),
                pltpu.VMEM((DM, FF), BF16),
                pltpu.VMEM((DM, FF), BF16),
                pltpu.VMEM((SLOTS, H, R, DH), BF16),
                pltpu.VMEM((NS, H, R), F32),
                pltpu.SemaphoreType.DMA((SLOTS,)),
                pltpu.SemaphoreType.DMA((13,)),
            ],
            compiler_params=pltpu.CompilerParams(
                vmem_limit_bytes=64 * 2**20,
                disable_bounds_checks=not checks,
                disable_semaphore_checks=not semchecks),
        )(A_x, A_k_cache, A_v_cache, A_wq, A_wo.T, B_w1, B_b1.reshape(FF // 128, 128), B_w2.T)

    return fn


_impl = make()


@jax.jit
def pallas_parallel_sum__mha_block_cached__dense_activation_mish__decode_kernel(
        A_x, A_k_cache, A_v_cache, A_wq, A_wo, B_x, B_w1, B_b1, B_w2):
    return _impl(A_x, A_k_cache, A_v_cache, A_wq, A_wo, B_x, B_w1, B_b1, B_w2)
```

```python
import functools

import jax
import jax.numpy as jnp
from jax import lax
from jax.experimental import pallas as pl
from jax.experimental.pallas import tpu as pltpu

KEYS = 128
PIECE = 64
AHEAD = 4
SLOTS = AHEAD + 1
QUEUE = 32
TILE = 8


def _dot(a, b):
    return jnp.dot(a, b, preferred_element_type=jnp.float32)


def _dot_t(a, b):
    return lax.dot_general(
        a, b, (((1,), (1,)), ((), ())), preferred_element_type=jnp.float32)


def _strided(n, stride):
    return [i for first in range(stride) for i in range(first, n, stride)]


class _Transfer:
    def __init__(self, src, dst, sem, row_tiles, cols):
        self.block = dst.at[pl.ds(TILE * min(row_tiles), TILE * len(row_tiles)), cols]
        self.sem = sem
        self.unstarted = len(row_tiles)
        self.pieces = [
            functools.partial(self._start, src, dst, (pl.ds(TILE * t, TILE), cols))
            for t in row_tiles
        ]

    def _start(self, src, dst, index, priority):
        copy = pltpu.make_async_copy(src.at[index], dst.at[index], self.sem)
        copy.start(priority=priority)
        self.unstarted -= 1

    def wait(self):
        assert self.unstarted == 0
        pltpu.make_async_copy(self.block, self.block, self.sem).wait()


class _Feeder:
    def __init__(self, priority_1, priority_0):
        self.lists = ((1, list(priority_1)), (0, list(priority_0)))

    def start(self, pairs):
        for _ in range(pairs):
            for priority, pieces in self.lists:
                if pieces:
                    pieces.pop(0)(priority)

    def finish(self):
        self.start(max(len(pieces) for _, pieces in self.lists))


def _body(x_hbm, k_hbm, v_hbm, wq_hbm, wo_hbm, w1_hbm, b1_hbm, w2_hbm, o_hbm,
          x_v, b1_v, o_v, wq_v, wo_v, w1_v, w2_v, s_v, rings, ring_sems, sems):
    _, heads, _, dh = k_hbm.shape
    d, ff = w1_v.shape
    steps = s_v.shape[0]
    tiles = d // TILE
    half = heads * dh // 2
    halves = (pl.ds(0, half), pl.ds(half, half))
    f32, bf16 = jnp.float32, jnp.bfloat16

    def cache_pieces(src, step, slot, parity):
        def start(h, offset, priority):
            row = step * KEYS + offset
            if not isinstance(row, int):
                row = pl.multiple_of(row, PIECE)
            pltpu.make_async_copy(
                src.at[0, h, pl.ds(row, PIECE)],
                rings[h].at[slot, pl.ds(offset, PIECE)],
                ring_sems[h].at[slot],
            ).start(priority=priority)

        return [functools.partial(start, h, offset)
                for offset in range(0, KEYS, PIECE)
                for h in range(parity, heads, 2)]

    def cache_feeder(src, step, slot):
        return _Feeder(cache_pieces(src, step, slot, 0), cache_pieces(src, step, slot, 1))

    def cache_wait(slot):
        for ring, sem in zip(rings, ring_sems):
            pltpu.make_async_copy(ring.at[slot], ring.at[slot], sem.at[slot]).wait()

    def next_slot(slot):
        return jnp.where(slot == SLOTS - 1, 0, slot + 1)

    wq = [_Transfer(wq_hbm, wq_v, sems.at[2 + i], _strided(tiles, 14), cols)
          for i, cols in enumerate(halves)]
    w1 = _Transfer(w1_hbm, w1_v, sems.at[4], _strided(tiles, 11), pl.ds(0, ff))
    cut = (tiles + QUEUE) // 2
    feed = _Feeder(
        wq[0].pieces[QUEUE:] + w1.pieces[:cut]
        + [p for s in range(AHEAD) for p in cache_pieces(k_hbm, s, s, 0)],
        wq[1].pieces + w1.pieces[cut:]
        + [p for s in range(AHEAD) for p in cache_pieces(k_hbm, s, s, 1)])
    for piece in wq[0].pieces[:QUEUE]:
        piece(1)
    x_copy = pltpu.make_async_copy(x_hbm, x_v, sems.at[0])
    b1_copy = pltpu.make_async_copy(b1_hbm, b1_v, sems.at[1])
    x_copy.start()
    b1_copy.start()
    feed.start(16)

    x_copy.wait()
    x = x_v[0].astype(f32)
    feed.start(2)
    centered = x - jnp.mean(x, axis=-1, keepdims=True)
    feed.start(2)
    var = jnp.mean(centered * centered, axis=-1, keepdims=True)
    feed.start(2)
    xn = jnp.broadcast_to(centered / jnp.sqrt(var + 1e-5), (heads, d)).astype(bf16)
    feed.start(2 * tiles - cut - 6)

    head_of_score = lax.broadcasted_iota(jnp.int32, (heads, KEYS), 0)
    head_of_value = lax.broadcasted_iota(jnp.int32, (heads, dh), 0)

    for w in wq:
        w.wait()
    q = jnp.zeros((heads, dh), f32)
    for h in range(heads):
        feed.start(2)
        q = jnp.where(head_of_value == h, _dot(xn, wq_v[:, h * dh:(h + 1) * dh]), q)
    q = (q * dh ** -0.5).astype(bf16)

    w1.wait()
    b1_copy.wait()
    b1 = b1_v[...].astype(f32)
    act = []
    for c in range(ff // 128):
        feed.start(1)
        z = _dot(xn, w1_v[:, c * 128:(c + 1) * 128]) + b1[c:c + 1, :]
        softplus = jnp.log1p(jnp.exp(-jnp.abs(z))) + jnp.where(z > 0, z, 0.0)
        act.append((z * jnp.tanh(softplus)).astype(bf16))
    act = jnp.concatenate(act, axis=1)
    feed.finish()

    def k_step(src, ahead, i, carry):
        slot, free, top = carry
        feed = cache_feeder(src, i + ahead, free)
        cache_wait(slot)
        s = jnp.zeros((heads, KEYS), f32)
        for h in range(heads):
            feed.start(1)
            s = jnp.where(head_of_score == h, _dot_t(q, rings[h][slot]), s)
        feed.finish()
        s_v[i] = s
        return next_slot(slot), slot, jnp.maximum(top, s)

    carry = (0, SLOTS - 1, jnp.full((heads, KEYS), -jnp.inf, f32))
    carry = lax.fori_loop(
        0, steps - AHEAD, functools.partial(k_step, k_hbm, AHEAD), carry)
    slot, free, top = lax.fori_loop(
        steps - AHEAD, steps, functools.partial(k_step, v_hbm, AHEAD - steps), carry)
    top = jnp.broadcast_to(jnp.max(top, axis=1, keepdims=True), (heads, KEYS))

    def v_step(i, slot, den, acc, feed):
        cache_wait(slot)
        p = jnp.exp(s_v[i] - top)
        p16 = p.astype(bf16)
        pv = jnp.zeros((heads, dh), f32)
        for h in range(heads):
            feed.start(1)
            pv = jnp.where(head_of_value == h, _dot(p16, rings[h][slot]), pv)
        return den + p, acc + pv

    def v_loop(i, carry):
        slot, free, den, acc = carry
        feed = cache_feeder(v_hbm, i + AHEAD, free)
        den, acc = v_step(i, slot, den, acc, feed)
        feed.finish()
        return next_slot(slot), slot, den, acc

    _, _, den, acc = lax.fori_loop(
        0, steps - AHEAD, v_loop,
        (slot, free, jnp.zeros((heads, KEYS), f32), jnp.zeros((heads, dh), f32)))

    wo = [_Transfer(wo_hbm, wo_v, sems.at[5 + i], _strided(tiles, 9), cols)
          for i, cols in enumerate(halves)]
    blocks = [(r, min(r + 128, d)) for r in range(0, d, 128)]
    w2 = [_Transfer(w2_hbm, w2_v, sems.at[7 + i], range(lo // TILE, hi // TILE), pl.ds(0, ff))
          for i, (lo, hi) in enumerate(blocks)]
    cut = tiles // 2 + len(w2[0].pieces)
    feed = _Feeder(
        wo[1].pieces[:cut] + [p for w in w2[1:] for p in w.pieces],
        wo[0].pieces + wo[1].pieces[cut:] + w2[0].pieces)
    for i in range(steps - AHEAD, steps):
        den, acc = v_step(i, (steps + i) % SLOTS, den, acc, feed)
    feed.start(2)
    o = acc / jnp.sum(den, axis=1, keepdims=True)
    o = [jnp.broadcast_to(o[h:h + 1, :], (heads, dh)).astype(bf16) for h in range(heads)]

    out = jnp.broadcast_to(x, (8, d))
    wo[0].wait()
    for h in range(heads // 2):
        feed.start(2)
        out = out + _dot_t(o[h], wo_v[:, h * dh:(h + 1) * dh])[:8]
    feed.finish()
    wo[1].wait()
    out = out + _dot_t(jnp.concatenate(o[heads // 2:], axis=1), wo_v[:, half:])[:8]
    for (lo, hi), w in zip(blocks, w2):
        w.wait()
        res = out[:, lo:hi] + _dot_t(act, w2_v[lo:hi, :])[:8]
        o_v[0, :, lo:hi] = res[:1].astype(o_v.dtype)

    out_copy = pltpu.make_async_copy(o_v, o_hbm, sems.at[0])
    out_copy.start()
    out_copy.wait()


@jax.jit
def pallas_parallel_sum__mha_block_cached__dense_activation_mish__decode_kernel(
    A_x: jax.Array,
    A_k_cache: jax.Array,
    A_v_cache: jax.Array,
    A_wq: jax.Array,
    A_wo: jax.Array,
    B_x: jax.Array,
    B_w1: jax.Array,
    B_b1: jax.Array,
    B_w2: jax.Array,
):
    del B_x
    _, heads, keys, dh = A_k_cache.shape
    d, ff = B_w1.shape
    assert A_x.shape == (1, 1, d) and A_k_cache.shape[0] == 1
    assert keys % KEYS == 0 and keys // KEYS >= AHEAD and ff % 128 == 0

    def kernel(*refs):
        pl.run_scoped(
            functools.partial(_body, *refs),
            [pltpu.SemaphoreType.DMA((SLOTS,)) for _ in range(heads)],
            pltpu.SemaphoreType.DMA((7 + pl.cdiv(d, 128),)),
        )

    hbm = pl.BlockSpec(memory_space=pltpu.HBM)
    return pl.pallas_call(
        kernel,
        out_shape=jax.ShapeDtypeStruct(A_x.shape, A_x.dtype),
        in_specs=[hbm] * 8,
        out_specs=hbm,
        scratch_shapes=[
            pltpu.VMEM(A_x.shape, A_x.dtype),
            pltpu.VMEM((ff // 128, 128), B_b1.dtype),
            pltpu.VMEM(A_x.shape, A_x.dtype),
            pltpu.VMEM((d, heads * dh), A_wq.dtype),
            pltpu.VMEM((d, heads * dh), A_wo.dtype),
            pltpu.VMEM((d, ff), B_w1.dtype),
            pltpu.VMEM((d, ff), B_w2.dtype),
            pltpu.VMEM((keys // KEYS, heads, KEYS), jnp.float32),
            [pltpu.VMEM((SLOTS, KEYS, dh), A_k_cache.dtype) for _ in range(heads)],
        ],
        compiler_params=pltpu.CompilerParams(vmem_limit_bytes=32 * 2**20),
    )(A_x, A_k_cache, A_v_cache, A_wq, A_wo.T, B_w1, B_b1.reshape(ff // 128, 128), B_w2.T)
```

```python
import functools

import jax
import jax.numpy as jnp
from jax import lax
from jax.experimental import pallas as pl
from jax.experimental.pallas import tpu as pltpu

KEYS = 128
PIECE = 64
AHEAD = 4
SLOTS = AHEAD + 1
QUEUE = 32
TILE = 8


def _dot(a, b):
    return jnp.dot(a, b, preferred_element_type=jnp.float32)


def _dot_t(a, b):
    return lax.dot_general(
        a, b, (((1,), (1,)), ((), ())), preferred_element_type=jnp.float32)


class _Transfer:
    def __init__(self, src, dst, sem, rows, cols, stride):
        self.block = dst.at[rows, cols]
        self.sem = sem
        self.unstarted = rows.size // TILE
        self.pieces = [
            functools.partial(
                self._start, src, dst, (pl.ds(rows.start + t * TILE, TILE), cols))
            for first in range(stride)
            for t in range(first, self.unstarted, stride)
        ]

    def _start(self, src, dst, index, priority):
        copy = pltpu.make_async_copy(src.at[index], dst.at[index], self.sem)
        copy.start(priority=priority)
        self.unstarted -= 1

    def wait(self):
        assert self.unstarted == 0
        pltpu.make_async_copy(self.block, self.block, self.sem).wait()


class _Feeder:
    def __init__(self, priority_1, priority_0):
        self.lists = ((1, list(priority_1)), (0, list(priority_0)))

    def start(self, pairs):
        for _ in range(pairs):
            for priority, pieces in self.lists:
                if pieces:
                    pieces.pop(0)(priority)

    def finish(self):
        self.start(max(len(pieces) for _, pieces in self.lists))


def _body(x_hbm, k_hbm, v_hbm, wq_hbm, wo_hbm, w1_hbm, b1_hbm, w2_hbm, o_hbm,
          x_v, b1_v, o_v, wq_v, wo_v, w1_v, w2_v, s_v, rings, ring_sems, sems):
    _, heads, _, dh = k_hbm.shape
    d, ff = w1_v.shape
    steps = s_v.shape[0]
    tiles = d // TILE
    half = heads * dh // 2
    halves = (pl.ds(0, half), pl.ds(half, half))
    f32, bf16 = jnp.float32, jnp.bfloat16

    def cache_copy(src, step, slot, h, offset):
        row = step * KEYS + offset
        if not isinstance(row, int):
            row = pl.multiple_of(row, PIECE)
        return pltpu.make_async_copy(
            src.at[0, h, pl.ds(row, PIECE)],
            rings[h].at[slot, pl.ds(offset, PIECE)],
            ring_sems.at[slot])

    def cache_pieces(src, step, slot, parity):
        def start(h, offset, priority):
            cache_copy(src, step, slot, h, offset).start(priority=priority)

        return [functools.partial(start, h, offset)
                for offset in range(0, KEYS, PIECE)
                for h in range(parity, heads, 2)]

    def cache_feeder(src, step, slot):
        return _Feeder(cache_pieces(src, step, slot, 0), cache_pieces(src, step, slot, 1))

    def cache_wait(src, step, slot):
        for offset in range(0, KEYS, PIECE):
            for h in range(heads):
                cache_copy(src, step, slot, h, offset).wait()

    def next_slot(slot):
        return jnp.where(slot == SLOTS - 1, 0, slot + 1)

    wq = [_Transfer(wq_hbm, wq_v, sems.at[2 + i], pl.ds(0, d), cols, stride=8)
          for i, cols in enumerate(halves)]
    w1 = _Transfer(w1_hbm, w1_v, sems.at[4], pl.ds(0, d), pl.ds(0, ff), stride=19)

    for piece in wq[0].pieces[:QUEUE]:
        piece(1)
    x_copy = pltpu.make_async_copy(x_hbm, x_v, sems.at[0])
    b1_copy = pltpu.make_async_copy(b1_hbm, b1_v, sems.at[1])
    x_copy.start()
    b1_copy.start()
    cut = (tiles + QUEUE) // 2
    _Feeder(wq[0].pieces[QUEUE:] + w1.pieces[:cut], wq[1].pieces + w1.pieces[cut:]).finish()
    feed = _Feeder(
        [p for s in range(AHEAD) for p in cache_pieces(k_hbm, s, s, 0)],
        [p for s in range(AHEAD) for p in cache_pieces(k_hbm, s, s, 1)])

    x_copy.wait()
    x = x_v[0].astype(f32)
    centered = x - jnp.mean(x, axis=-1, keepdims=True)
    var = jnp.mean(centered * centered, axis=-1, keepdims=True)
    xn = jnp.broadcast_to(centered / jnp.sqrt(var + 1e-5), (heads, d)).astype(bf16)
    feed.start(heads)

    head_of_score = lax.broadcasted_iota(jnp.int32, (heads, KEYS), 0)
    head_of_value = lax.broadcasted_iota(jnp.int32, (heads, dh), 0)

    q = jnp.zeros((heads, dh), f32)
    for h in range(heads):
        if h % (heads // 2) == 0:
            wq[h // (heads // 2)].wait()
        feed.start(2)
        q = jnp.where(head_of_value == h, _dot(xn, wq_v[:, h * dh:(h + 1) * dh]), q)
    q = (q * dh ** -0.5).astype(bf16)

    w1.wait()
    b1_copy.wait()
    b1 = b1_v[...].astype(f32)
    act = []
    for c in range(ff // 128):
        feed.start(1)
        z = _dot(xn, w1_v[:, c * 128:(c + 1) * 128]) + b1[c:c + 1, :]
        softplus = jnp.log1p(jnp.exp(-jnp.abs(z))) + jnp.where(z > 0, z, 0.0)
        act.append((z * jnp.tanh(softplus)).astype(bf16))
    act = jnp.concatenate(act, axis=1)
    feed.finish()

    def k_step(src, ahead, i, carry):
        slot, free, top = carry
        feed = cache_feeder(src, i + ahead, free)
        cache_wait(k_hbm, i, slot)
        s = jnp.zeros((heads, KEYS), f32)
        for h in range(heads):
            feed.start(1)
            s = jnp.where(head_of_score == h, _dot_t(q, rings[h][slot]), s)
        feed.finish()
        s_v[i] = s
        return next_slot(slot), slot, jnp.maximum(top, s)

    carry = (0, SLOTS - 1, jnp.full((heads, KEYS), -jnp.inf, f32))
    carry = lax.fori_loop(
        0, steps - AHEAD, functools.partial(k_step, k_hbm, AHEAD), carry)
    slot, free, top = lax.fori_loop(
        steps - AHEAD, steps, functools.partial(k_step, v_hbm, AHEAD - steps), carry)
    top = jnp.broadcast_to(jnp.max(top, axis=1, keepdims=True), (heads, KEYS))

    def v_step(i, slot, den, acc, feed):
        cache_wait(v_hbm, i, slot)
        p = jnp.exp(s_v[i] - top)
        p16 = p.astype(bf16)
        pv = jnp.zeros((heads, dh), f32)
        for h in range(heads):
            feed.start(1)
            pv = jnp.where(head_of_value == h, _dot(p16, rings[h][slot]), pv)
        return den + p, acc + pv

    def v_loop(i, carry):
        slot, free, den, acc = carry
        feed = cache_feeder(v_hbm, i + AHEAD, free)
        den, acc = v_step(i, slot, den, acc, feed)
        feed.finish()
        return next_slot(slot), slot, den, acc

    _, _, den, acc = lax.fori_loop(
        0, steps - AHEAD, v_loop,
        (slot, free, jnp.zeros((heads, KEYS), f32), jnp.zeros((heads, dh), f32)))

    wo = [_Transfer(wo_hbm, wo_v, sems.at[5 + i], pl.ds(0, d), cols, stride=8)
          for i, cols in enumerate(halves)]
    blocks = [(r, min(r + 128, d)) for r in range(0, d, 128)]
    w2 = [_Transfer(w2_hbm, w2_v, sems.at[7 + i], pl.ds(lo, hi - lo), pl.ds(0, ff), stride=1)
          for i, (lo, hi) in enumerate(blocks)]
    cut = tiles // 2 + len(w2[0].pieces)
    feed = _Feeder(
        wo[1].pieces[:cut] + [p for w in w2[1:] for p in w.pieces],
        wo[0].pieces + wo[1].pieces[cut:] + w2[0].pieces)
    for i in range(steps - AHEAD, steps):
        den, acc = v_step(i, (steps + i) % SLOTS, den, acc, feed)
    feed.start(2)
    o = acc / jnp.sum(den, axis=1, keepdims=True)
    o = [jnp.broadcast_to(o[h:h + 1, :], (heads, dh)).astype(bf16) for h in range(heads)]

    out = jnp.broadcast_to(x, (8, d))
    wo[0].wait()
    for h in range(heads // 2):
        feed.start(2)
        out = out + _dot_t(o[h], wo_v[:, h * dh:(h + 1) * dh])[:8]
    feed.finish()
    wo[1].wait()
    out = out + _dot_t(jnp.concatenate(o[heads // 2:], axis=1), wo_v[:, half:])[:8]
    for (lo, hi), w in zip(blocks, w2):
        w.wait()
        res = out[:, lo:hi] + _dot_t(act, w2_v[lo:hi, :])[:8]
        o_v[0, :, lo:hi] = res[:1].astype(o_v.dtype)

    out_copy = pltpu.make_async_copy(o_v, o_hbm, sems.at[0])
    out_copy.start()
    out_copy.wait()


@jax.jit
def pallas_parallel_sum__mha_block_cached__dense_activation_mish__decode_kernel(
    A_x: jax.Array,
    A_k_cache: jax.Array,
    A_v_cache: jax.Array,
    A_wq: jax.Array,
    A_wo: jax.Array,
    B_x: jax.Array,
    B_w1: jax.Array,
    B_b1: jax.Array,
    B_w2: jax.Array,
):
    del B_x
    _, heads, keys, dh = A_k_cache.shape
    d, ff = B_w1.shape
    assert A_x.shape == (1, 1, d) and A_k_cache.shape[0] == 1
    assert keys % KEYS == 0 and keys // KEYS >= AHEAD and ff % 128 == 0
    assert d % (2 * TILE) == 0 and heads % 2 == 0

    def kernel(*refs):
        pl.run_scoped(
            functools.partial(_body, *refs),
            pltpu.SemaphoreType.DMA((SLOTS,)),
            pltpu.SemaphoreType.DMA((7 + pl.cdiv(d, 128),)),
        )

    hbm = pl.BlockSpec(memory_space=pltpu.HBM)
    return pl.pallas_call(
        kernel,
        out_shape=jax.ShapeDtypeStruct(A_x.shape, A_x.dtype),
        in_specs=[hbm] * 8,
        out_specs=hbm,
        scratch_shapes=[
            pltpu.VMEM(A_x.shape, A_x.dtype),
            pltpu.VMEM((ff // 128, 128), B_b1.dtype),
            pltpu.VMEM(A_x.shape, A_x.dtype),
            pltpu.VMEM((d, heads * dh), A_wq.dtype),
            pltpu.VMEM((d, heads * dh), A_wo.dtype),
            pltpu.VMEM((d, ff), B_w1.dtype),
            pltpu.VMEM((d, ff), B_w2.dtype),
            pltpu.VMEM((keys // KEYS, heads, KEYS), jnp.float32),
            [pltpu.VMEM((SLOTS, KEYS, dh), A_k_cache.dtype) for _ in range(heads)],
        ],
        compiler_params=pltpu.CompilerParams(vmem_limit_bytes=32 * 2**20),
    )(A_x, A_k_cache, A_v_cache, A_wq, A_wo.T, B_w1, B_b1.reshape(ff // 128, 128), B_w2.T)
```
